```python
import jax
import jax.numpy as jnp

def _softmax(x, axis=-1):
    return jax.nn.softmax(x, axis=axis)
def _gelu(x):
    return jax.nn.gelu(x, approximate=True)
def _silu(x):
    return jax.nn.silu(x)
def _sigmoid(x):
    return jax.nn.sigmoid(x)
def _layernorm(x, axis=-1, eps=1e-5):
    m = jnp.mean(x, axis=axis, keepdims=True)
    v = jnp.var(x, axis=axis, keepdims=True)
    return (x - m) / jnp.sqrt(v + eps)
def _scatter_add(tgt, idx, src, axis=0):
    return tgt.at[idx].add(src)
def _segment_sum(src, seg, n):
    return jax.ops.segment_sum(src, seg, n)
class _Rng:
    def __init__(self, key):
        self._k = key
    def _next(self):
        self._k, sub = jax.random.split(self._k)
        return sub
    def normal(self, shape):
        return jax.random.normal(self._next(), shape, dtype=jnp.bfloat16)
    def randint(self, lo, hi, shape):
        return jax.random.randint(self._next(), shape, lo, hi, dtype=jnp.int32)
    def uniform(self, shape, lo=0.0, hi=1.0):
        return jax.random.uniform(self._next(), shape, jnp.bfloat16, lo, hi)
    def permutation(self, n):
        return jax.random.permutation(self._next(), n)


kernel_name = 'sequential_preLN__compressed_kv_cla__moe_arch_mod__prompt'

def setup_inputs():
    _rng = _Rng(jax.random.key(int.from_bytes(__import__("os").urandom(4), "little")))
    _w = (lambda a: (lambda t: t.astype(jnp.bfloat16) if jnp.issubdtype(t.dtype, jnp.floating) else t)(jnp.asarray(a)))
    def _A_setup():
        B, H, Sq, Sk, D, M = 1, 32, 2048, 2048, 128, 1024
        Dc = 4 * D
        return {
            "x": _w((lambda *s: _rng.normal(s) * 0.05)(B, Sq, M)),
            "c_kv": _w((lambda *s: _rng.normal(s) * 0.05)(B, Sk, Dc)),
            "w_q": _w((lambda *s: _rng.normal(s) * 0.05)(M, H, D) * (M ** -0.5)),
            "w_uk": _w((lambda *s: _rng.normal(s) * 0.05)(Dc, H, D) * (Dc ** -0.5)),
            "w_uv": _w((lambda *s: _rng.normal(s) * 0.05)(Dc, H, D) * (Dc ** -0.5)),
            "w_o": _w((lambda *s: _rng.normal(s) * 0.05)(H, D, M) * ((H * D) ** -0.5)),
        }
    _A_in = _A_setup()

    def _B_setup():
        B, S, D, F, C = 1, 2048, 1024, 3584, 2
        return {
            "x": _w((lambda *s: _rng.normal(s) * 0.05)(B, S, D)),
            "w_r": _w((lambda *s: _rng.normal(s) * 0.05)(D)),
            "w_gate": _w((lambda *s: _rng.normal(s) * 0.05)(D, F)),
            "w_up": _w((lambda *s: _rng.normal(s) * 0.05)(D, F)),
            "w_down": _w((lambda *s: _rng.normal(s) * 0.05)(F, D)),
        }
    _B_in = _B_setup()

    return {
        "A_x": _A_in["x"],
        "A_c_kv": _A_in["c_kv"],
        "A_w_q": _A_in["w_q"],
        "A_w_uk": _A_in["w_uk"],
        "A_w_uv": _A_in["w_uv"],
        "A_w_o": _A_in["w_o"],
        "B_x": _B_in["x"],
        "B_w_r": _B_in["w_r"],
        "B_w_gate": _B_in["w_gate"],
        "B_w_up": _B_in["w_up"],
        "B_w_down": _B_in["w_down"],
    }

def reference(A_x, A_c_kv, A_w_q, A_w_uk, A_w_uv, A_w_o, B_x, B_w_r, B_w_gate, B_w_up, B_w_down):
    def _A_ref(x, c_kv, w_q, w_uk, w_uv, w_o):
        B, Sq, M = x.shape[0], x.shape[1], x.shape[2]
        Sk = c_kv.shape[1]
        H, D = w_q.shape[1], w_q.shape[2]
        q = jnp.einsum("bqm,mhd->bhqd", x, w_q)
        k = jnp.einsum("bkc,chd->bhkd", c_kv, w_uk)
        v = jnp.einsum("bkc,chd->bhkd", c_kv, w_uv)
        scores = jnp.einsum("bhqd,bhkd->bhqk", q, k) * (D ** -0.5)
        off = Sk - Sq
        qi = jnp.arange(Sq)[:, None]
        kj = jnp.arange(Sk)[None, :]
        cmask = kj <= (qi + off)
        scores = jnp.where(cmask[None, None], scores, -1e9)
        p = _softmax(scores, axis=-1)
        ctx = jnp.einsum("bhqk,bhkd->bhqd", p, v)
        return jnp.einsum("bhqd,hdm->bqm", ctx, w_o)

    def _B_ref(x, w_r, w_gate, w_up, w_down):
        B, S, D = x.shape
        C = 2
        r = x @ w_r
        idx = jnp.argsort(-r, axis=-1)[:, :C]
        idx_e = jnp.repeat(idx.reshape(B, C, 1), D, axis=2)
        x_sel = jnp.take_along_axis(x, idx_e, axis=1)
        g = _silu(x_sel @ w_gate)
        u = x_sel @ w_up
        y = (g * u) @ w_down
        r_sel = _sigmoid(jnp.take_along_axis(r, idx, axis=1))
        y = y * r_sel.reshape(B, C, 1)
        b_off = (jnp.arange(B) * S).reshape(B, 1)
        flat_idx = (idx + b_off).reshape(B * C)
        zero = (x * 0.0).reshape(B * S, D)
        upd = _scatter_add(zero, flat_idx, y.reshape(B * C, D), axis=0)
        return x + upd.reshape(B, S, D)

    x = A_x
    h = x + _A_ref(_layernorm(x, axis=-1), A_c_kv, A_w_q, A_w_uk, A_w_uv, A_w_o)
    h2 = h + _B_ref(_layernorm(h, axis=-1), B_w_r, B_w_gate, B_w_up, B_w_down)
    return h2
```

```python
import functools

import jax
import jax.numpy as jnp
import numpy as np
import jax.experimental.pallas as pl
import jax.experimental.pallas.tpu as pltpu

S = 2048
M = 1024
DC = 512
H = 32
D = 128
F = 3584
BQ = 256
NQ = S // BQ
LOG2E = 1.4426950408889634
QSCALE = float(D ** -0.5) * LOG2E
NEG = -1e9 * LOG2E
EPS = 1e-5

f32 = jnp.float32
bf16 = jnp.bfloat16


def _rb(x):
    return x.astype(bf16).astype(f32)


def _ln_bf16(x):
    mean = jnp.mean(x, axis=-1, keepdims=True)
    xc = x - mean
    var = jnp.mean(xc * xc, axis=-1, keepdims=True)
    d = _rb(x - _rb(mean))
    s = _rb(jnp.sqrt(_rb(_rb(var) + np.float32(EPS))))
    return d * (1.0 / s)


def _relayout(raw_ref, dst_ref, rows):
    r32 = raw_ref.bitcast(jnp.uint32)

    def body(c, carry):
        slab = r32.at[pl.ds(pl.multiple_of(c * (128 * 16), 128 * 16), 128 * 16), :]
        for j in range(H // 2):
            w32 = slab[pl.ds(j, 128, stride=H // 2), :]
            lo = pltpu.bitcast(w32 << 16, f32).astype(bf16)
            hi = pltpu.bitcast(w32 & jnp.uint32(0xFFFF0000), f32).astype(bf16)
            r0 = pl.multiple_of(c * 128, 128)
            dst_ref[j, pl.ds(r0, 128), 0:D] = lo
            dst_ref[j, pl.ds(r0, 128), D:2 * D] = hi
        return carry

    jax.lax.fori_loop(0, rows // 128, body, 0)


def _nt(a, b):
    return jax.lax.dot_general(a, b, (((1,), (1,)), ((), ())), preferred_element_type=f32)


def _mm(a, b):
    return jnp.dot(a, b, preferred_element_type=f32)


def _kernel(x_hbm, c_hbm, wq_hbm, wuk_hbm, wuv_hbm, wo_hbm, wr_ref, wg_hbm, wu_hbm, wd_hbm,
            out_ref,
            x_v, c_v, wq_v, wuk_v, wuv_v, wo_v, wg_v, wu_v, wd_v,
            wq2_v, wk2_v, wv2_v, xn_v, q_v, k_v, v_v, ctx_v, s_v, acc_v, sems):
    cps = [
        pltpu.make_async_copy(c_hbm, c_v, sems.at[0]),
        pltpu.make_async_copy(x_hbm, x_v, sems.at[1]),
        pltpu.make_async_copy(wuk_hbm, wuk_v, sems.at[2]),
        pltpu.make_async_copy(wuv_hbm, wuv_v, sems.at[3]),
        pltpu.make_async_copy(wq_hbm, wq_v, sems.at[4]),
        pltpu.make_async_copy(wo_hbm, wo_v, sems.at[5]),
        pltpu.make_async_copy(wg_hbm, wg_v, sems.at[6]),
        pltpu.make_async_copy(wu_hbm, wu_v, sems.at[7]),
        pltpu.make_async_copy(wd_hbm, wd_v, sems.at[8]),
    ]
    for c in cps:
        c.start()
    cps[1].wait()
    for i in range(NQ):
        rows = pl.ds(i * BQ, BQ)
        xn_v[rows, :] = _ln_bf16(x_v[rows, :].astype(f32)).astype(bf16)
        acc_v[rows, :] = jnp.zeros((BQ, M), f32)
    cps[0].wait()
    cps[2].wait()
    cps[3].wait()
    cps[4].wait()
    cps[5].wait()
    _relayout(wuk_v, wk2_v, DC)
    _relayout(wuv_v, wv2_v, DC)
    _relayout(wq_v, wq2_v, M)

    row = jax.lax.broadcasted_iota(jnp.int32, (BQ, BQ), 0)
    col = jax.lax.broadcasted_iota(jnp.int32, (BQ, BQ), 1)
    causal = col <= row

    def pair_body(j, carry):
        wq = wq2_v[j]
        wk = wk2_v[j]
        wv = wv2_v[j]
        q_v[...] = (_mm(xn_v[...], wq) * QSCALE).astype(bf16)
        k_v[...] = _mm(c_v[...], wk).astype(bf16)
        v_v[...] = _mm(c_v[...], wv).astype(bf16)
        for hh in range(2):
            hc = pl.ds(hh * D, D)
            for i in range(NQ):
                q = q_v[pl.ds(i * BQ, BQ), hc]
                m = None
                for t in range(i + 1):
                    s = _nt(q, k_v[pl.ds(t * BQ, BQ), hc])
                    if t == i:
                        s = jnp.where(causal, s, NEG)
                    s_v[:, pl.ds(t * BQ, BQ)] = s
                    mt = jnp.maximum(s[:, :128], s[:, 128:])
                    m = mt if m is None else jnp.maximum(m, mt)
                mrow = jnp.max(m, axis=1, keepdims=True)
                l = None
                acc = None
                for t in range(i + 1):
                    p = jnp.exp2(s_v[:, pl.ds(t * BQ, BQ)] - mrow)
                    lt = p[:, :128] + p[:, 128:]
                    l = lt if l is None else l + lt
                    pv = _mm(p.astype(bf16), v_v[pl.ds(t * BQ, BQ), hc])
                    acc = pv if acc is None else acc + pv
                lrow = jnp.sum(l, axis=1, keepdims=True)
                ctx_v[pl.ds(i * BQ, BQ), hc] = (acc * (1.0 / lrow)).astype(bf16)
        wo = wo_v[pl.ds(2 * j, 2)].reshape(2 * D, M)
        acc_v[...] += _mm(ctx_v[...], wo)
        return carry

    jax.lax.fori_loop(0, H // 2, pair_body, 0)

    wr = jnp.broadcast_to(wr_ref[...], (16, M))
    r_parts = []
    for i in range(NQ):
        rows = pl.ds(i * BQ, BQ)
        h = _rb(x_v[rows, :].astype(f32) + _rb(acc_v[rows, :]))
        hn = _ln_bf16(h).astype(bf16)
        acc_v[rows, :] = h
        xn_v[rows, :] = hn
        r_parts.append(_nt(wr, hn))
    r = _rb(jnp.concatenate(r_parts, axis=1))
    r = r[:8]
    tok = jax.lax.broadcasted_iota(jnp.int32, (8, S), 1)
    m1 = jnp.max(r, axis=1, keepdims=True)
    i1 = jnp.min(jnp.where(r == m1, tok, S), axis=1, keepdims=True)
    r2 = jnp.where(tok == i1, -jnp.inf, r)
    m2 = jnp.max(r2, axis=1, keepdims=True)
    i2 = jnp.min(jnp.where(r2 == m2, tok, S), axis=1, keepdims=True)
    sub = jax.lax.broadcasted_iota(jnp.int32, (8, S), 0)
    isel = jnp.where(sub == 0, i1, i2)
    onehot = jnp.where((tok == isel) & (sub < 2), 1.0, 0.0).astype(f32)
    onehot = jnp.concatenate([onehot, jnp.zeros_like(onehot)], axis=0).astype(bf16)
    xs = _mm(onehot, xn_v[...]).astype(bf16)
    cps[6].wait()
    cps[7].wait()
    cps[8].wait()
    g = _rb(_mm(xs, wg_v[...]))
    g = _rb(g * _rb(jax.nn.sigmoid(g)))
    u = _rb(_mm(xs, wu_v[...]))
    a = (g * u).astype(bf16)
    y = _rb(_mm(a, wd_v[...]))
    sub1 = jax.lax.broadcasted_iota(jnp.int32, (16, 1), 0)
    rsel = jnp.where(sub1 == 0, m1[0:1, :], m2[0:1, :])
    y = _rb(y * _rb(jax.nn.sigmoid(rsel)))
    y1 = y[0:1, :]
    y2 = y[1:2, :]
    i1s = i1[0:1, :]
    i2s = i2[0:1, :]
    for i in range(NQ):
        rows = pl.ds(i * BQ, BQ)
        rid = jax.lax.broadcasted_iota(jnp.int32, (BQ, 1), 0) + i * BQ
        upd = jnp.where(rid == i1s, y1, 0.0) + jnp.where(rid == i2s, y2, 0.0)
        hn = xn_v[rows, :].astype(f32)
        out_ref[rows, :] = (acc_v[rows, :] + _rb(hn + upd)).astype(bf16)


@jax.jit
def pallas_sequential_preLN__compressed_kv_cla__moe_arch_mod__prompt_kernel(
        A_x, A_c_kv, A_w_q, A_w_uk, A_w_uv, A_w_o, B_x, B_w_r, B_w_gate, B_w_up, B_w_down):
    any_spec = pl.BlockSpec(memory_space=pl.ANY)
    vmem_spec = pl.BlockSpec(memory_space=pltpu.VMEM)
    out = pl.pallas_call(
        _kernel,
        out_shape=jax.ShapeDtypeStruct((S, M), bf16),
        in_specs=[any_spec] * 6 + [vmem_spec] + [any_spec] * 3,
        out_specs=vmem_spec,
        scratch_shapes=[
            pltpu.VMEM((S, M), bf16),
            pltpu.VMEM((S, DC), bf16),
            pltpu.VMEM((M * H, D), bf16),
            pltpu.VMEM((DC * H, D), bf16),
            pltpu.VMEM((DC * H, D), bf16),
            pltpu.VMEM((H, D, M), bf16),
            pltpu.VMEM((M, F), bf16),
            pltpu.VMEM((M, F), bf16),
            pltpu.VMEM((F, M), bf16),
            pltpu.VMEM((H // 2, M, 2 * D), bf16),
            pltpu.VMEM((H // 2, DC, 2 * D), bf16),
            pltpu.VMEM((H // 2, DC, 2 * D), bf16),
            pltpu.VMEM((S, M), bf16),
            pltpu.VMEM((S, 2 * D), bf16),
            pltpu.VMEM((S, 2 * D), bf16),
            pltpu.VMEM((S, 2 * D), bf16),
            pltpu.VMEM((S, 2 * D), bf16),
            pltpu.VMEM((BQ, S), f32),
            pltpu.VMEM((S, M), f32),
            pltpu.SemaphoreType.DMA((9,)),
        ],
        compiler_params=pltpu.CompilerParams(vmem_limit_bytes=120 * 1024 * 1024),
    )(A_x.reshape(S, M), A_c_kv.reshape(S, DC), A_w_q.reshape(M * H, D),
      A_w_uk.reshape(DC * H, D), A_w_uv.reshape(DC * H, D), A_w_o,
      B_w_r.reshape(1, M), B_w_gate, B_w_up, B_w_down)
    return out.reshape(1, S, M)
```

```python
import functools

import jax
import jax.numpy as jnp
import numpy as np
import jax.experimental.pallas as pl
import jax.experimental.pallas.tpu as pltpu

S = 2048
M = 1024
DC = 512
H = 32
D = 128
F = 3584
NP = H // 2
BQ = 256
NQ = S // BQ
LOG2E = 1.4426950408889634
QSCALE = float(D ** -0.5) * LOG2E
NEG = -1e9 * LOG2E
EPS = 1e-5
CH = 128 * H
TC = 512
LR = 128

f32 = jnp.float32
bf16 = jnp.bfloat16


def _rb(x):
    return x.astype(bf16).astype(f32)


def _ln_bf16(x):
    mean = jnp.mean(x, axis=-1, keepdims=True)
    xc = x - mean
    var = jnp.mean(xc * xc, axis=-1, keepdims=True)
    d = _rb(x - _rb(mean))
    s = _rb(jnp.sqrt(_rb(_rb(var) + np.float32(EPS))))
    return d * (1.0 / s)


def _nt(a, b):
    return jax.lax.dot_general(a, b, (((1,), (1,)), ((), ())), preferred_element_type=f32)


def _mm(a, b):
    return jnp.dot(a, b, preferred_element_type=f32)


BIG = 3e38


def _tie(lhs, dep):
    c = dep[:8] + dep[8:] if dep.shape[0] == 16 else dep
    w = lhs.shape[1]
    c = functools.reduce(lambda a, b: a + b, [c[:, n:n + w] for n in range(0, c.shape[1], w)])
    h32 = pltpu.bitcast(lhs[:16], jnp.uint32)
    h32 = jnp.where(c != c, jnp.uint32(0x7FC07FC0), h32)
    return jnp.concatenate([pltpu.bitcast(h32, bf16), lhs[16:]], axis=0)


def _relayout(stg_ref, slot, dst_ref, row0, pairs=range(NP)):
    slab = stg_ref.bitcast(jnp.uint32).at[slot]
    rows = pl.ds(pl.multiple_of(row0, 128), 128)
    for j in pairs:
        w32 = slab[pl.ds(j, 128, stride=NP), :]
        lo = pltpu.bitcast(w32 << 16, f32).astype(bf16)
        hi = pltpu.bitcast(w32 & jnp.uint32(0xFFFF0000), f32).astype(bf16)
        dst_ref[j, rows, 0:D] = lo
        dst_ref[j, rows, D:2 * D] = hi


def _kernel(x_hbm, c_hbm, wq_hbm, wuk_hbm, wuv_hbm, wo_hbm, wr_ref, wg_hbm, wu_hbm, wd_hbm,
            out_hbm,
            x_v, c_v, stg, wo_v, wg_v, wu_v, wd_v,
            w2_v, xn_v, q_v, k_v, v_v, ctx_v, acc_v, o_v, r_v, pt_v,
            sem_c, sem_x, sem_w, sem_big, sem_o, sem_p):
    def c_copy(t):
        r = pl.ds(pl.multiple_of(t * TC, TC), TC)
        return pltpu.make_async_copy(c_hbm.at[r], c_v.at[r], sem_c.at[t])

    def x_copy(t):
        r = pl.ds(pl.multiple_of(t * LR, LR), LR)
        return pltpu.make_async_copy(x_hbm.at[r], x_v.at[r], sem_x.at[t])

    def w_copy(src, k, slot):
        r = pl.ds(pl.multiple_of(k * CH, CH), CH)
        return pltpu.make_async_copy(src.at[r], stg.at[slot], sem_w.at[slot])

    big = [
        pltpu.make_async_copy(wo_hbm, wo_v, sem_big.at[0]),
        pltpu.make_async_copy(wg_hbm, wg_v, sem_big.at[1]),
        pltpu.make_async_copy(wu_hbm, wu_v, sem_big.at[2]),
        pltpu.make_async_copy(wd_hbm, wd_v, sem_big.at[3]),
    ]

    for k in range(4):
        w_copy(wuk_hbm, k, k).start()
    c_copy(0).start()
    x_copy(0).start()

    def a_body(k, carry):
        w_copy(wuk_hbm, k, k).wait()
        _relayout(stg, k, w2_v, k * 128)
        w_copy(wuv_hbm, k, k).start()
        return carry

    if True:
        jax.lax.fori_loop(0, 4, a_body, 0)
    for t in range(1, 3):
        x_copy(t).start()
    c_copy(1).start()

    def b_step(it, slot, dst_row):
        rows = pl.ds(pl.multiple_of((it // 4) * TC, TC), TC)
        cc = c_v[rows, :]
        dep = None
        for jj in range(4):
            p = (it % 4) * 4 + jj
            for n in range(2):
                kr = pl.ds(pl.multiple_of((it // 4) * TC + n * 256, 256), 256)
                lhs = cc[n * 256:(n + 1) * 256]
                if dep is not None:
                    lhs = _tie(lhs, dep)
                k_v[p, kr, :] = _mm(lhs, w2_v[p, 0:DC, :]).astype(bf16)
                u = jj * 2 + n
                lr = pl.ds(pl.multiple_of(it * LR + u * 16, 16), 16)
                dep = _ln_bf16(x_v[lr, :].astype(f32))
                xn_v[lr, :] = dep.astype(bf16)
                if dst_row is not None:
                    _relayout(stg, slot, w2_v, dst_row, range(2 * u, 2 * u + 2))

    def b_body(src_next, kofs, dst0, it0):
        def body(i, carry):
            it = it0 + i
            slot = i % 4

            @pl.when(it % 4 == 0)
            def _():
                c_copy(it // 4).wait()

                @pl.when(it // 4 + 2 < S // TC)
                def _():
                    c_copy(it // 4 + 2).start()

            x_copy(it).wait()

            @pl.when(it + 3 < S // LR)
            def _():
                x_copy(it + 3).start()

            if dst0 is not None:
                w_copy(wq_hbm, 0, slot).wait()
            b_step(it, slot, None if dst0 is None else dst0 + i * 128)
            if dst0 is not None:
                if src_next is not None:
                    w_copy(src_next, kofs + i, slot).start()
            return carry
        return body

    if True:
        jax.lax.fori_loop(0, 4, b_body(wq_hbm, 0, DC, 0), 0)
    if True:
        jax.lax.fori_loop(0, 4, b_body(wq_hbm, 4, 2 * DC, 4), 0)
    if True:
        jax.lax.fori_loop(0, 4, b_body(None, 0, 2 * DC + 512, 8), 0)
    if True:
        jax.lax.fori_loop(0, 4, b_body(None, 0, None, 12), 0)

    for c in big:
        c.start()
    tri = (jax.lax.broadcasted_iota(jnp.int32, (128, 128), 1)
           <= jax.lax.broadcasted_iota(jnp.int32, (128, 128), 0))

    def pair_body(j, carry):
        wq = w2_v[j, 2 * DC:, :]
        wv = w2_v[j, DC:2 * DC, :]

        def proj(i):
            rows = pl.ds(i * BQ, BQ)
            q_v[rows, :] = (_mm(xn_v[rows, :], wq) * QSCALE).astype(bf16)
            v_v[rows, :] = _mm(c_v[rows, :], wv).astype(bf16)

        HB = BQ // 2

        def qk(hh, i):
            hc = pl.ds(hh * D, D)
            q = q_v[pl.ds(i * BQ, BQ), hc]
            top, bot = [], []
            for t in range(i):
                s = _nt(q, k_v[j, pl.ds(t * BQ, BQ), hc])
                top += [s[:HB, :128], s[:HB, 128:]]
                bot += [s[HB:, :128], s[HB:, 128:]]
            s = _nt(q, k_v[j, pl.ds(i * BQ, 128), hc])
            top.append(jnp.where(tri, s[:HB], NEG))
            bot.append(s[HB:])
            s = _nt(q[HB:], k_v[j, pl.ds(i * BQ + 128, 128), hc])
            bot.append(jnp.where(tri, s, NEG))
            mt = jnp.max(functools.reduce(jnp.maximum, top), axis=1, keepdims=True)
            mb_ = jnp.max(functools.reduce(jnp.maximum, bot), axis=1, keepdims=True)
            return top, bot, jnp.broadcast_to(mt, (HB, 128)), jnp.broadcast_to(mb_, (HB, 128))

        def pv(hh, i, st, prev):
            hc = pl.ds(hh * D, D)
            top, bot, mt, mb_ = st
            m = jnp.concatenate([mt, mb_], axis=0)
            l = acc = None
            accs = []
            for t in range(i):
                if t == 0:
                    w = prev
                elif t == 1:
                    w = l
                else:
                    w = l + accs[-2]
                mm_ = m if w is None else jnp.maximum(m, w - BIG)
                p0 = jnp.exp2(jnp.concatenate([top[2 * t], bot[2 * t]], axis=0) - mm_)
                p1 = jnp.exp2(jnp.concatenate([top[2 * t + 1], bot[2 * t + 1]], axis=0) - mm_)
                lt = p0 + p1
                l = lt if l is None else l + lt
                p = jnp.concatenate([p0, p1], axis=1).astype(bf16)
                o = _mm(p, v_v[pl.ds(t * BQ, BQ), hc])
                acc = o if acc is None else acc + o
                accs.append(acc)
            w = prev if i == 0 else (l if i == 1 else l + accs[-2])
            mm_ = m if w is None else jnp.maximum(m, w - BIG)
            p0 = jnp.exp2(jnp.concatenate([top[-1], bot[-2]], axis=0) - mm_)
            p1 = jnp.exp2(bot[-1] - mm_[HB:])
            o0 = _mm(p0.astype(bf16), v_v[pl.ds(i * BQ, 128), hc])
            o1 = _mm(p1.astype(bf16), v_v[pl.ds(i * BQ + 128, 128), hc])
            l = p0 if l is None else l + p0
            acc = o0 if acc is None else acc + o0
            l = jnp.concatenate([l[:HB], l[HB:] + p1], axis=0)
            acc = jnp.concatenate([acc[:HB], acc[HB:] + o1], axis=0)
            lrow = jnp.sum(l, axis=1, keepdims=True)
            o = acc * (1.0 / lrow)
            ctx_v[j, pl.ds(i * BQ, BQ), hc] = o.astype(bf16)
            return o

        blocks = [(hh, i) for i in range(NQ) for hh in range(2)]
        proj(0)
        st = qk(*blocks[0])
        prev = None
        for n, blk in enumerate(blocks):
            if blk[0] == 0 and blk[1] + 1 < NQ:
                proj(blk[1] + 1)
            nxt = qk(*blocks[n + 1]) if n + 1 < len(blocks) else None
            prev = pv(*blk, st, prev)
            st = nxt
        return carry

    if True:
        jax.lax.fori_loop(0, NP, pair_body, 0)

    big[0].wait()
    wr = jnp.broadcast_to(wr_ref[...].reshape(1, M), (16, M))

    def o_copy(i):
        r = pl.ds(pl.multiple_of(i * BQ, BQ), BQ)
        return pltpu.make_async_copy(o_v.at[r], out_hbm.at[r], sem_o.at[i])

    def epi(i, u):
        rows = pl.ds(pl.multiple_of(i * BQ + u * 16, 16), 16)
        acc = acc_v[i % 2, pl.ds(u * 16, 16), :]
        h = _rb(x_v[rows, :].astype(f32) + _rb(acc))
        hn = _ln_bf16(h).astype(bf16)
        x_v[rows, :] = h.astype(bf16)
        xn_v[rows, :] = hn
        o = h + hn.astype(f32)
        o_v[rows, :] = o.astype(bf16)
        return o

    def epi_done(i):
        rows = pl.ds(pl.multiple_of(i * BQ, BQ), BQ)
        r_v[i] = _rb(_nt(wr, xn_v[rows, :])[:8])
        o_copy(i).start()

    def d_step(i, with_epi):
        rows = pl.ds(pl.multiple_of(i * BQ, BQ), BQ)
        acc = dep = None
        for p in range(NP):
            lhs = ctx_v[p, rows, :]
            if dep is not None:
                lhs = _tie(lhs, dep)
            t = _mm(lhs, wo_v[p])
            acc = t if acc is None else acc + t
            if with_epi:
                dep = epi(i - 1, p)
        acc_v[i % 2] = acc
        if with_epi:
            epi_done(i - 1)

    def d_body(i, carry):
        d_step(i, True)
        return carry

    if True:
        d_step(0, False)
        jax.lax.fori_loop(1, NQ, d_body, 0)
        for u in range(NP):
            epi(NQ - 1, u)
        epi_done(NQ - 1)

    r = jnp.concatenate([r_v[i] for i in range(NQ)], axis=1)
    tok = jax.lax.broadcasted_iota(jnp.int32, (8, S), 1)
    m1 = jnp.max(r, axis=1, keepdims=True)
    i1v = jnp.min(jnp.where(r == m1, tok, S), axis=1, keepdims=True)
    r2 = jnp.where(tok == i1v, -jnp.inf, r)
    m2 = jnp.max(r2, axis=1, keepdims=True)
    i2v = jnp.min(jnp.where(r2 == m2, tok, S), axis=1, keepdims=True)
    i1 = jnp.clip(jnp.max(i1v), 0, S - 1)
    i2 = jnp.clip(jnp.max(i2v), 0, S - 1)
    g1 = pl.multiple_of((i1 // 16) * 16, 16)
    g2 = pl.multiple_of((i2 // 16) * 16, 16)
    xs = jnp.concatenate([xn_v[pl.ds(g1, 16), :], xn_v[pl.ds(g2, 16), :]], axis=0)
    for c in big[1:]:
        c.wait()
    g = _rb(_mm(xs, wg_v[...]))
    g = _rb(g * _rb(jax.nn.sigmoid(g)))
    u = _rb(_mm(xs, wu_v[...]))
    a = (g * u).astype(bf16)
    y = _rb(_mm(a, wd_v[...]))
    s1 = _rb(jax.nn.sigmoid(m1[0:1, :]))
    s2 = _rb(jax.nn.sigmoid(m2[0:1, :]))
    rid = jax.lax.broadcasted_iota(jnp.int32, (16, 1), 0)
    for n, gbase in enumerate((g1, g2)):
        yy = y[n * 16:(n + 1) * 16, :]
        upd = (jnp.where(rid + gbase == i1, _rb(yy * s1), 0.0)
               + jnp.where(rid + gbase == i2, _rb(yy * s2), 0.0))
        hh_ = x_v[pl.ds(gbase, 16), :].astype(f32)
        hn_ = xs[n * 16:(n + 1) * 16, :].astype(f32)
        pt_v[n] = (hh_ + _rb(hn_ + upd)).astype(bf16)
    for i in range(NQ):
        o_copy(i).wait()
    for n, gbase in enumerate((g1, g2)):
        cp = pltpu.make_async_copy(pt_v.at[n], out_hbm.at[pl.ds(gbase, 16)], sem_p.at[n])
        cp.start()
        cp.wait()


@jax.jit
def pallas_sequential_preLN__compressed_kv_cla__moe_arch_mod__prompt_kernel(
        A_x, A_c_kv, A_w_q, A_w_uk, A_w_uv, A_w_o, B_x, B_w_r, B_w_gate, B_w_up, B_w_down):
    any_spec = pl.BlockSpec(memory_space=pl.ANY)
    vmem_spec = pl.BlockSpec(memory_space=pltpu.VMEM)
    out = pl.pallas_call(
        _kernel,
        out_shape=jax.ShapeDtypeStruct((S, M), bf16),
        in_specs=[any_spec] * 6 + [vmem_spec] + [any_spec] * 3,
        out_specs=any_spec,
        scratch_shapes=[
            pltpu.VMEM((S, M), bf16),
            pltpu.VMEM((S, DC), bf16),
            pltpu.VMEM((4, CH, D), bf16),
            pltpu.VMEM((NP, 2 * D, M), bf16),
            pltpu.VMEM((M, F), bf16),
            pltpu.VMEM((M, F), bf16),
            pltpu.VMEM((F, M), bf16),
            pltpu.VMEM((NP, 2 * DC + M, 2 * D), bf16),
            pltpu.VMEM((S, M), bf16),
            pltpu.VMEM((S, 2 * D), bf16),
            pltpu.VMEM((NP, S, 2 * D), bf16),
            pltpu.VMEM((S, 2 * D), bf16),
            pltpu.VMEM((NP, S, 2 * D), bf16),
            pltpu.VMEM((2, BQ, M), f32),
            pltpu.VMEM((S, M), bf16),
            pltpu.VMEM((NQ, 8, BQ), f32),
            pltpu.VMEM((2, 16, M), bf16),
            pltpu.SemaphoreType.DMA((S // TC,)),
            pltpu.SemaphoreType.DMA((S // LR,)),
            pltpu.SemaphoreType.DMA((4,)),
            pltpu.SemaphoreType.DMA((4,)),
            pltpu.SemaphoreType.DMA((NQ,)),
            pltpu.SemaphoreType.DMA((2,)),
        ],
        compiler_params=pltpu.CompilerParams(vmem_limit_bytes=120 * 1024 * 1024),
    )(A_x.reshape(S, M), A_c_kv.reshape(S, DC), A_w_q.reshape(M * H, D),
      A_w_uk.reshape(DC * H, D), A_w_uv.reshape(DC * H, D), A_w_o.reshape(NP, 2 * D, M),
      B_w_r, B_w_gate, B_w_up, B_w_down)
    return out.reshape(1, S, M)
```

```python
import functools

import jax
import jax.numpy as jnp
import numpy as np
import jax.experimental.pallas as pl
import jax.experimental.pallas.tpu as pltpu

S = 2048
M = 1024
DC = 512
H = 32
D = 128
F = 3584
NP = H // 2
BQ = 256
NQ = S // BQ
LOG2E = 1.4426950408889634
QSCALE = float(D ** -0.5) * LOG2E
NEG = -1e9 * LOG2E
EPS = 1e-5
CH = 128 * H
TC = 512
LR = 128

f32 = jnp.float32
bf16 = jnp.bfloat16


def _rb(x):
    return x.astype(bf16).astype(f32)


def _ln_bf16(x):
    mean = jnp.mean(x, axis=-1, keepdims=True)
    xc = x - mean
    var = jnp.mean(xc * xc, axis=-1, keepdims=True)
    d = _rb(x - _rb(mean))
    s = _rb(jnp.sqrt(_rb(_rb(var) + np.float32(EPS))))
    return d * (1.0 / s)


def _nt(a, b):
    return jax.lax.dot_general(a, b, (((1,), (1,)), ((), ())), preferred_element_type=f32)


def _mm(a, b):
    return jnp.dot(a, b, preferred_element_type=f32)


BIG = 3e38


def _tie(lhs, dep):
    c = dep[:8] + dep[8:] if dep.shape[0] == 16 else dep
    w = lhs.shape[1]
    c = functools.reduce(lambda a, b: a + b, [c[:, n:n + w] for n in range(0, c.shape[1], w)])
    h32 = pltpu.bitcast(lhs[:16], jnp.uint32)
    h32 = jnp.where(c != c, jnp.uint32(0x7FC07FC0), h32)
    return jnp.concatenate([pltpu.bitcast(h32, bf16), lhs[16:]], axis=0)


def _relayout(stg_ref, slot, dst_ref, row0, pairs=range(NP)):
    slab = stg_ref.bitcast(jnp.uint32).at[slot]
    rows = pl.ds(pl.multiple_of(row0, 128), 128)
    for j in pairs:
        w32 = slab[pl.ds(j, 128, stride=NP), :]
        lo = pltpu.bitcast(w32 << 16, f32).astype(bf16)
        hi = pltpu.bitcast(w32 & jnp.uint32(0xFFFF0000), f32).astype(bf16)
        dst_ref[j, rows, 0:D] = lo
        dst_ref[j, rows, D:2 * D] = hi


def _kernel(x_hbm, c_hbm, wq_hbm, wuk_hbm, wuv_hbm, wo_hbm, wr_ref, wg_hbm, wu_hbm, wd_hbm,
            out_hbm,
            x_v, c_v, stg, wo_v, wg_v, wu_v, wd_v,
            w2_v, xn_v, q_v, k_v, v_v, ctx_v, acc_v, o_v, r_v, pt_v,
            sem_c, sem_x, sem_w, sem_big, sem_o, sem_p):
    def c_copy(t):
        r = pl.ds(pl.multiple_of(t * TC, TC), TC)
        return pltpu.make_async_copy(c_hbm.at[r], c_v.at[r], sem_c.at[t])

    def x_copy(t):
        r = pl.ds(pl.multiple_of(t * LR, LR), LR)
        return pltpu.make_async_copy(x_hbm.at[r], x_v.at[r], sem_x.at[t])

    def w_copy(src, k, slot):
        r = pl.ds(pl.multiple_of(k * CH, CH), CH)
        return pltpu.make_async_copy(src.at[r], stg.at[slot], sem_w.at[slot])

    big = [
        pltpu.make_async_copy(wo_hbm, wo_v, sem_big.at[0]),
        pltpu.make_async_copy(wg_hbm, wg_v, sem_big.at[1]),
        pltpu.make_async_copy(wu_hbm, wu_v, sem_big.at[2]),
        pltpu.make_async_copy(wd_hbm, wd_v, sem_big.at[3]),
    ]

    for k in range(4):
        w_copy(wuk_hbm, k, k).start()

    for k in range(4):
        w_copy(wuk_hbm, k, k).wait()
        if k == 0:
            c_copy(0).start()
            x_copy(0).start()
        _relayout(stg, k, w2_v, k * 128)
    for t in range(1, 3):
        x_copy(t).start()
    c_copy(1).start()

    def b_step(it, slot, dst_row):
        rows = pl.ds(pl.multiple_of((it // 4) * TC, TC), TC)
        cc = c_v[rows, :]
        dep = None
        for jj in range(4):
            p = (it % 4) * 4 + jj
            for n in range(2):
                kr = pl.ds(pl.multiple_of((it // 4) * TC + n * 256, 256), 256)
                lhs = cc[n * 256:(n + 1) * 256]
                if dep is not None:
                    lhs = _tie(lhs, dep)
                k_v[p, kr, :] = _mm(lhs, w2_v[p, 0:DC, :]).astype(bf16)
                u = jj * 2 + n
                lr = pl.ds(pl.multiple_of(it * LR + u * 16, 16), 16)
                dep = _ln_bf16(x_v[lr, :].astype(f32))
                xn_v[lr, :] = dep.astype(bf16)
                if dst_row is not None:
                    _relayout(stg, slot, w2_v, dst_row, range(2 * u, 2 * u + 2))

    def b_body(src_next, kofs, dst0, it0):
        def body(i, carry):
            it = it0 + i
            slot = i % 4

            @pl.when(it % 4 == 0)
            def _():
                c_copy(it // 4).wait()

                @pl.when(it // 4 + 2 < S // TC)
                def _():
                    c_copy(it // 4 + 2).start()

            x_copy(it).wait()

            @pl.when(it + 3 < S // LR)
            def _():
                x_copy(it + 3).start()

            if dst0 is not None:
                w_copy(wq_hbm, 0, slot).wait()
            b_step(it, slot, None if dst0 is None else dst0 + i * 128)
            if src_next is not None:
                w_copy(src_next, kofs + i, slot).start()
            return carry
        return body

    jax.lax.fori_loop(0, 4, b_body(wuv_hbm, 0, None, 0), 0)
    jax.lax.fori_loop(0, 4, b_body(wq_hbm, 0, DC, 4), 0)
    jax.lax.fori_loop(0, 4, b_body(wq_hbm, 4, 2 * DC, 8), 0)
    jax.lax.fori_loop(0, 4, b_body(None, 0, 2 * DC + 512, 12), 0)

    for c in big:
        c.start()
    tri = (jax.lax.broadcasted_iota(jnp.int32, (128, 128), 1)
           <= jax.lax.broadcasted_iota(jnp.int32, (128, 128), 0))

    def pair_body(j, carry):
        wq = w2_v[j, 2 * DC:, :]
        wv = w2_v[j, DC:2 * DC, :]

        def proj(i):
            rows = pl.ds(i * BQ, BQ)
            q_v[rows, :] = (_mm(xn_v[rows, :], wq) * QSCALE).astype(bf16)
            v_v[rows, :] = _mm(c_v[rows, :], wv).astype(bf16)

        HB = BQ // 2

        def qk(hh, i):
            hc = pl.ds(hh * D, D)
            q = q_v[pl.ds(i * BQ, BQ), hc]
            top, bot = [], []
            for t in range(i):
                s = _nt(q, k_v[j, pl.ds(t * BQ, BQ), hc])
                top += [s[:HB, :128], s[:HB, 128:]]
                bot += [s[HB:, :128], s[HB:, 128:]]
            s = _nt(q, k_v[j, pl.ds(i * BQ, 128), hc])
            top.append(jnp.where(tri, s[:HB], NEG))
            bot.append(s[HB:])
            s = _nt(q[HB:], k_v[j, pl.ds(i * BQ + 128, 128), hc])
            bot.append(jnp.where(tri, s, NEG))
            mt = jnp.max(functools.reduce(jnp.maximum, top), axis=1, keepdims=True)
            mb_ = jnp.max(functools.reduce(jnp.maximum, bot), axis=1, keepdims=True)
            return top, bot, jnp.broadcast_to(mt, (HB, 128)), jnp.broadcast_to(mb_, (HB, 128))

        def pv(hh, i, st, prev):
            hc = pl.ds(hh * D, D)
            top, bot, mt, mb_ = st
            m = jnp.concatenate([mt, mb_], axis=0)
            l = acc = None
            accs = []
            for t in range(i):
                if t == 0:
                    w = prev
                elif t <= 2:
                    w = l
                else:
                    w = l + accs[-3]
                mm_ = m if w is None else jnp.maximum(m, w - BIG)
                p0 = jnp.exp2(jnp.concatenate([top[2 * t], bot[2 * t]], axis=0) - mm_)
                p1 = jnp.exp2(jnp.concatenate([top[2 * t + 1], bot[2 * t + 1]], axis=0) - mm_)
                lt = p0 + p1
                l = lt if l is None else l + lt
                p = jnp.concatenate([p0, p1], axis=1).astype(bf16)
                o = _mm(p, v_v[pl.ds(t * BQ, BQ), hc])
                acc = o if acc is None else acc + o
                accs.append(acc)
            w = prev if i == 0 else (l if i <= 2 else l + accs[-3])
            mm_ = m if w is None else jnp.maximum(m, w - BIG)
            p0 = jnp.exp2(jnp.concatenate([top[-1], bot[-2]], axis=0) - mm_)
            p1 = jnp.exp2(bot[-1] - mm_[HB:])
            o0 = _mm(p0.astype(bf16), v_v[pl.ds(i * BQ, 128), hc])
            o1 = _mm(p1.astype(bf16), v_v[pl.ds(i * BQ + 128, 128), hc])
            l = p0 if l is None else l + p0
            acc = o0 if acc is None else acc + o0
            l = jnp.concatenate([l[:HB], l[HB:] + p1], axis=0)
            acc = jnp.concatenate([acc[:HB], acc[HB:] + o1], axis=0)
            lrow = jnp.sum(l, axis=1, keepdims=True)
            o = acc * (1.0 / lrow)
            ctx_v[j, pl.ds(i * BQ, BQ), hc] = o.astype(bf16)
            return o

        blocks = [(hh, i) for i in range(NQ) for hh in range(2)]
        proj(0)
        st = qk(*blocks[0])
        prev = None
        for n, blk in enumerate(blocks):
            if blk[0] == 0 and blk[1] + 1 < NQ:
                proj(blk[1] + 1)
            nxt = qk(*blocks[n + 1]) if n + 1 < len(blocks) else None
            prev = pv(*blk, st, prev)
            st = nxt
        return carry

    jax.lax.fori_loop(0, NP, pair_body, 0)

    big[0].wait()
    wr = jnp.broadcast_to(wr_ref[...].reshape(1, M), (16, M))

    def o_copy(i):
        r = pl.ds(pl.multiple_of(i * BQ, BQ), BQ)
        return pltpu.make_async_copy(o_v.at[r], out_hbm.at[r], sem_o.at[i])

    def epi(i, u):
        rows = pl.ds(pl.multiple_of(i * BQ + u * 16, 16), 16)
        acc = acc_v[i % 2, pl.ds(u * 16, 16), :]
        h = _rb(x_v[rows, :].astype(f32) + _rb(acc))
        hn = _ln_bf16(h).astype(bf16)
        x_v[rows, :] = h.astype(bf16)
        xn_v[rows, :] = hn
        o = h + hn.astype(f32)
        o_v[rows, :] = o.astype(bf16)
        return o

    def epi_done(i):
        rows = pl.ds(pl.multiple_of(i * BQ, BQ), BQ)
        r_v[i] = _rb(_nt(wr, xn_v[rows, :])[:8])
        o_copy(i).start()

    def d_step(i, with_epi):
        rows = pl.ds(pl.multiple_of(i * BQ, BQ), BQ)
        acc = dep = None
        for p in range(NP):
            lhs = ctx_v[p, rows, :]
            if dep is not None:
                lhs = _tie(lhs, dep)
            t = _mm(lhs, wo_v[p])
            acc = t if acc is None else acc + t
            if with_epi:
                dep = epi(i - 1, p)
        acc_v[i % 2] = acc
        if with_epi:
            epi_done(i - 1)

    def d_body(i, carry):
        d_step(i, True)
        return carry

    d_step(0, False)
    jax.lax.fori_loop(1, NQ, d_body, 0)
    for u in range(NP):
        epi(NQ - 1, u)
    epi_done(NQ - 1)

    r = jnp.concatenate([r_v[i] for i in range(NQ)], axis=1)
    tok = jax.lax.broadcasted_iota(jnp.int32, (8, S), 1)
    m1 = jnp.max(r, axis=1, keepdims=True)
    i1v = jnp.min(jnp.where(r == m1, tok, S), axis=1, keepdims=True)
    r2 = jnp.where(tok == i1v, -jnp.inf, r)
    m2 = jnp.max(r2, axis=1, keepdims=True)
    i2v = jnp.min(jnp.where(r2 == m2, tok, S), axis=1, keepdims=True)
    i1 = jnp.clip(jnp.max(i1v), 0, S - 1)
    i2 = jnp.clip(jnp.max(i2v), 0, S - 1)
    g1 = pl.multiple_of((i1 // 16) * 16, 16)
    g2 = pl.multiple_of((i2 // 16) * 16, 16)
    xs = jnp.concatenate([xn_v[pl.ds(g1, 16), :], xn_v[pl.ds(g2, 16), :]], axis=0)
    for c in big[1:]:
        c.wait()
    g = _rb(_mm(xs, wg_v[...]))
    g = _rb(g * _rb(jax.nn.sigmoid(g)))
    u = _rb(_mm(xs, wu_v[...]))
    a = (g * u).astype(bf16)
    y = _rb(_mm(a, wd_v[...]))
    s1 = _rb(jax.nn.sigmoid(m1[0:1, :]))
    s2 = _rb(jax.nn.sigmoid(m2[0:1, :]))
    rid = jax.lax.broadcasted_iota(jnp.int32, (16, 1), 0)
    for n, gbase in enumerate((g1, g2)):
        yy = y[n * 16:(n + 1) * 16, :]
        upd = (jnp.where(rid + gbase == i1, _rb(yy * s1), 0.0)
               + jnp.where(rid + gbase == i2, _rb(yy * s2), 0.0))
        hh_ = x_v[pl.ds(gbase, 16), :].astype(f32)
        hn_ = xs[n * 16:(n + 1) * 16, :].astype(f32)
        pt_v[n] = (hh_ + _rb(hn_ + upd)).astype(bf16)
    for i in range(NQ):
        o_copy(i).wait()
    for n, gbase in enumerate((g1, g2)):
        cp = pltpu.make_async_copy(pt_v.at[n], out_hbm.at[pl.ds(gbase, 16)], sem_p.at[n])
        cp.start()
        cp.wait()


@jax.jit
def pallas_sequential_preLN__compressed_kv_cla__moe_arch_mod__prompt_kernel(
        A_x, A_c_kv, A_w_q, A_w_uk, A_w_uv, A_w_o, B_x, B_w_r, B_w_gate, B_w_up, B_w_down):
    any_spec = pl.BlockSpec(memory_space=pl.ANY)
    vmem_spec = pl.BlockSpec(memory_space=pltpu.VMEM)
    out = pl.pallas_call(
        _kernel,
        out_shape=jax.ShapeDtypeStruct((S, M), bf16),
        in_specs=[any_spec] * 6 + [vmem_spec] + [any_spec] * 3,
        out_specs=any_spec,
        scratch_shapes=[
            pltpu.VMEM((S, M), bf16),
            pltpu.VMEM((S, DC), bf16),
            pltpu.VMEM((4, CH, D), bf16),
            pltpu.VMEM((NP, 2 * D, M), bf16),
            pltpu.VMEM((M, F), bf16),
            pltpu.VMEM((M, F), bf16),
            pltpu.VMEM((F, M), bf16),
            pltpu.VMEM((NP, 2 * DC + M, 2 * D), bf16),
            pltpu.VMEM((S, M), bf16),
            pltpu.VMEM((S, 2 * D), bf16),
            pltpu.VMEM((NP, S, 2 * D), bf16),
            pltpu.VMEM((S, 2 * D), bf16),
            pltpu.VMEM((NP, S, 2 * D), bf16),
            pltpu.VMEM((2, BQ, M), f32),
            pltpu.VMEM((S, M), bf16),
            pltpu.VMEM((NQ, 8, BQ), f32),
            pltpu.VMEM((2, 16, M), bf16),
            pltpu.SemaphoreType.DMA((S // TC,)),
            pltpu.SemaphoreType.DMA((S // LR,)),
            pltpu.SemaphoreType.DMA((4,)),
            pltpu.SemaphoreType.DMA((4,)),
            pltpu.SemaphoreType.DMA((NQ,)),
            pltpu.SemaphoreType.DMA((2,)),
        ],
        compiler_params=pltpu.CompilerParams(vmem_limit_bytes=120 * 1024 * 1024),
    )(A_x.reshape(S, M), A_c_kv.reshape(S, DC), A_w_q.reshape(M * H, D),
      A_w_uk.reshape(DC * H, D), A_w_uv.reshape(DC * H, D), A_w_o.reshape(NP, 2 * D, M),
      B_w_r, B_w_gate, B_w_up, B_w_down)
    return out.reshape(1, S, M)
```

```python
import functools

import jax
import jax.numpy as jnp
import numpy as np
import jax.experimental.pallas as pl
import jax.experimental.pallas.tpu as pltpu

S = 2048
M = 1024
DC = 512
H = 32
D = 128
F = 3584
NP = H // 2
BQ = 256
NQ = S // BQ
LOG2E = 1.4426950408889634
QSCALE = float(D ** -0.5) * LOG2E
NEG = -1e9 * LOG2E
EPS = 1e-5
CH = 128 * H
TC = 512
LR = 128

f32 = jnp.float32
bf16 = jnp.bfloat16


def _rb(x):
    return x.astype(bf16).astype(f32)


def _ln_bf16(x):
    mean = jnp.mean(x, axis=-1, keepdims=True)
    xc = x - mean
    var = jnp.mean(xc * xc, axis=-1, keepdims=True)
    d = _rb(x - _rb(mean))
    s = _rb(jnp.sqrt(_rb(_rb(var) + np.float32(EPS))))
    return d * (1.0 / s)


def _nt(a, b):
    return jax.lax.dot_general(a, b, (((1,), (1,)), ((), ())), preferred_element_type=f32)


def _mm(a, b):
    return jnp.dot(a, b, preferred_element_type=f32)


def _after(x, w):
    return jnp.where(w != w, w, x)


def _tie(lhs, dep):
    c = dep[:8] + dep[8:] if dep.shape[0] == 16 else dep
    w = lhs.shape[1]
    c = functools.reduce(lambda a, b: a + b, [c[:, n:n + w] for n in range(0, c.shape[1], w)])
    h32 = pltpu.bitcast(lhs[:16], jnp.uint32)
    h32 = jnp.where(c != c, jnp.uint32(0x7FC07FC0), h32)
    return jnp.concatenate([pltpu.bitcast(h32, bf16), lhs[16:]], axis=0)


def _relayout(stg_ref, slot, dst_ref, row0, pairs=range(NP)):
    slab = stg_ref.bitcast(jnp.uint32).at[slot]
    rows = pl.ds(pl.multiple_of(row0, 128), 128)
    for j in pairs:
        w32 = slab[pl.ds(j, 128, stride=NP), :]
        lo = pltpu.bitcast(w32 << 16, f32).astype(bf16)
        hi = pltpu.bitcast(w32 & jnp.uint32(0xFFFF0000), f32).astype(bf16)
        dst_ref[j, rows, 0:D] = lo
        dst_ref[j, rows, D:2 * D] = hi


def _kernel(x_hbm, c_hbm, wq_hbm, wuk_hbm, wuv_hbm, wo_hbm, wr_ref, wg_hbm, wu_hbm, wd_hbm,
            out_hbm,
            x_v, c_v, stg, wo_v, wg_v, wu_v, wd_v,
            w2_v, xn_v, q0_v, q_v, k_v, v_v, ctx_v, acc_v, o_v, r_v, pt_v,
            sem_c, sem_x, sem_w, sem_big, sem_o, sem_p):
    def c_copy(t):
        r = pl.ds(pl.multiple_of(t * TC, TC), TC)
        return pltpu.make_async_copy(c_hbm.at[r], c_v.at[r], sem_c.at[t])

    def x_copy(t):
        r = pl.ds(pl.multiple_of(t * LR, LR), LR)
        return pltpu.make_async_copy(x_hbm.at[r], x_v.at[r], sem_x.at[t])

    def w_copy(src, k, slot):
        r = pl.ds(pl.multiple_of(k * CH, CH), CH)
        return pltpu.make_async_copy(src.at[r], stg.at[slot], sem_w.at[slot])

    big = [
        pltpu.make_async_copy(wo_hbm, wo_v, sem_big.at[0]),
        pltpu.make_async_copy(wg_hbm, wg_v, sem_big.at[1]),
        pltpu.make_async_copy(wu_hbm, wu_v, sem_big.at[2]),
        pltpu.make_async_copy(wd_hbm, wd_v, sem_big.at[3]),
    ]

    for k in range(4):
        w_copy(wuk_hbm, k, k).start()

    for k in range(4):
        w_copy(wuk_hbm, k, k).wait()
        if k == 0:
            c_copy(0).start()
            x_copy(0).start()
        _relayout(stg, k, w2_v, k * 128)
    for t in range(1, 3):
        x_copy(t).start()
    c_copy(1).start()

    def b_step(it, slot, dst_row):
        rows = pl.ds(pl.multiple_of((it // 4) * TC, TC), TC)
        cc = c_v[rows, :]
        dep = kprev = None
        for jj in range(4):
            p = (it % 4) * 4 + jj
            for n in range(2):
                kr = pl.ds(pl.multiple_of((it // 4) * TC + n * 256, 256), 256)
                lhs = cc[n * 256:(n + 1) * 256]
                if dep is not None:
                    lhs = _tie(lhs, dep)
                kk = _mm(lhs, w2_v[p, 0:DC, :])
                k_v[p, kr, :] = kk.astype(bf16)
                u = jj * 2 + n
                lr = pl.ds(pl.multiple_of(it * LR + u * 16, 16), 16)
                xr = x_v[lr, :].astype(f32)
                if kprev is not None:
                    xr = _after(xr, jnp.concatenate([kprev] * 4, axis=1))
                kprev = kk[:16]
                dep = _ln_bf16(xr)
                xn_v[lr, :] = dep.astype(bf16)
                if dst_row is not None:
                    _relayout(stg, slot, w2_v, dst_row, range(2 * u, 2 * u + 2))

    def b_body(src_next, kofs, dst0, it0):
        def body(i, carry):
            it = it0 + i
            slot = i % 4

            @pl.when(it % 4 == 0)
            def _():
                c_copy(it // 4).wait()

                @pl.when(it // 4 + 2 < S // TC)
                def _():
                    c_copy(it // 4 + 2).start()

            x_copy(it).wait()

            @pl.when(it + 3 < S // LR)
            def _():
                x_copy(it + 3).start()

            if dst0 is not None:
                w_copy(wq_hbm, 0, slot).wait()
            b_step(it, slot, None if dst0 is None else dst0 + i * 128)
            if src_next is not None:
                w_copy(src_next, kofs + i, slot).start()
            return carry
        return body

    jax.lax.fori_loop(0, 4, b_body(wuv_hbm, 0, None, 0), 0)
    jax.lax.fori_loop(0, 4, b_body(wq_hbm, 0, DC, 4), 0)
    jax.lax.fori_loop(0, 4, b_body(wq_hbm, 4, 2 * DC, 8), 0)
    jax.lax.fori_loop(0, 4, b_body(None, 0, 2 * DC + 512, 12), 0)

    for c in big:
        c.start()
    tri = (jax.lax.broadcasted_iota(jnp.int32, (128, 128), 1)
           <= jax.lax.broadcasted_iota(jnp.int32, (128, 128), 0))

    def q_first(p, half):
        cols = pl.ds(half * D, D)
        q0_v[:, cols] = (_mm(xn_v[0:BQ, :], w2_v[p, 2 * DC:, cols]) * QSCALE).astype(bf16)

    q_first(0, 0)
    q_first(0, 1)

    def pair_body(j, carry):
        wq = w2_v[j, 2 * DC:, :]
        wv = w2_v[j, DC:2 * DC, :]

        def proj(i):
            rows = pl.ds(i * BQ, BQ)
            if i > 0:
                q_v[rows, :] = (_mm(xn_v[rows, :], wq) * QSCALE).astype(bf16)
            v_v[rows, :] = _mm(c_v[rows, :], wv).astype(bf16)

        HB = BQ // 2

        def qk(hh, i):
            hc = pl.ds(hh * D, D)
            q = q_v[pl.ds(i * BQ, BQ), hc] if i > 0 else q0[:, hh * D:(hh + 1) * D]
            top, bot = [], []
            for t in range(i):
                s = _nt(q, k_v[j, pl.ds(t * BQ, BQ), hc])
                top += [s[:HB, :128], s[:HB, 128:]]
                bot += [s[HB:, :128], s[HB:, 128:]]
            s = _nt(q, k_v[j, pl.ds(i * BQ, 128), hc])
            top.append(jnp.where(tri, s[:HB], NEG))
            bot.append(s[HB:])
            s = _nt(q[HB:], k_v[j, pl.ds(i * BQ + 128, 128), hc])
            bot.append(jnp.where(tri, s, NEG))
            mt = jnp.max(functools.reduce(jnp.maximum, top), axis=1, keepdims=True)
            mb_ = jnp.max(functools.reduce(jnp.maximum, bot), axis=1, keepdims=True)
            return top, bot, jnp.broadcast_to(mt, (HB, 128)), jnp.broadcast_to(mb_, (HB, 128))

        def pv(hh, i, st, prev):
            hc = pl.ds(hh * D, D)
            top, bot, mt, mb_ = st
            m = jnp.concatenate([mt, mb_], axis=0)
            l = acc = None
            accs = []
            for t in range(i):
                if t == 0:
                    w = prev
                elif t <= 2:
                    w = l
                else:
                    w = l + accs[-3]
                mm_ = m if w is None else _after(m, w)
                p0 = jnp.exp2(jnp.concatenate([top[2 * t], bot[2 * t]], axis=0) - mm_)
                p1 = jnp.exp2(jnp.concatenate([top[2 * t + 1], bot[2 * t + 1]], axis=0) - mm_)
                lt = p0 + p1
                l = lt if l is None else l + lt
                p = jnp.concatenate([p0, p1], axis=1).astype(bf16)
                o = _mm(p, v_v[pl.ds(t * BQ, BQ), hc])
                acc = o if acc is None else acc + o
                accs.append(acc)
            w = prev if i == 0 else (l if i <= 2 else l + accs[-3])
            mm_ = m if w is None else _after(m, w)
            p0 = jnp.exp2(jnp.concatenate([top[-1], bot[-2]], axis=0) - mm_)
            p1 = jnp.exp2(bot[-1] - mm_[HB:])
            o0 = _mm(p0.astype(bf16), v_v[pl.ds(i * BQ, 128), hc])
            o1 = _mm(p1.astype(bf16), v_v[pl.ds(i * BQ + 128, 128), hc])
            l = p0 if l is None else l + p0
            acc = o0 if acc is None else acc + o0
            l = jnp.concatenate([l[:HB], l[HB:] + p1], axis=0)
            acc = jnp.concatenate([acc[:HB], acc[HB:] + o1], axis=0)
            lrow = jnp.sum(l, axis=1, keepdims=True)
            o = acc * (1.0 / lrow)
            ctx_v[j, pl.ds(i * BQ, BQ), hc] = o.astype(bf16)
            return o

        q0 = q0_v[...]
        jn = jnp.minimum(j + 1, NP - 1)
        blocks = [(hh, i) for i in range(NQ) for hh in range(2)]
        proj(0)
        st = qk(*blocks[0])
        prev = None
        for n, blk in enumerate(blocks):
            if blk[0] == 0 and blk[1] + 1 < NQ:
                proj(blk[1] + 1)
            nxt = qk(*blocks[n + 1]) if n + 1 < len(blocks) else None
            if nxt is None:
                q_first(jn, 0)
            prev = pv(*blk, st, prev)
            st = nxt
        q_first(jn, 1)
        return carry

    jax.lax.fori_loop(0, NP, pair_body, 0)

    big[0].wait()
    wr = jnp.broadcast_to(wr_ref[...].reshape(1, M), (16, M))

    def o_copy(i):
        r = pl.ds(pl.multiple_of(i * BQ, BQ), BQ)
        return pltpu.make_async_copy(o_v.at[r], out_hbm.at[r], sem_o.at[i])

    def epi(i, u, after=None):
        rows = pl.ds(pl.multiple_of(i * BQ + u * 16, 16), 16)
        acc = acc_v[i % 2, pl.ds(u * 16, 16), :]
        if after is not None:
            acc = _after(acc, after)
        h = _rb(x_v[rows, :].astype(f32) + _rb(acc))
        hn = _ln_bf16(h).astype(bf16)
        x_v[rows, :] = h.astype(bf16)
        xn_v[rows, :] = hn
        o = h + hn.astype(f32)
        o_v[rows, :] = o.astype(bf16)
        return o

    def epi_done(i):
        rows = pl.ds(pl.multiple_of(i * BQ, BQ), BQ)
        r_v[i] = _rb(_nt(wr, xn_v[rows, :])[:8])
        o_copy(i).start()

    def d_step(i, with_epi):
        rows = pl.ds(pl.multiple_of(i * BQ, BQ), BQ)
        acc = dep = tprev = None
        for p in range(NP):
            lhs = ctx_v[p, rows, :]
            if dep is not None:
                lhs = _tie(lhs, dep)
            t = _mm(lhs, wo_v[p])
            acc = t if acc is None else acc + t
            if with_epi:
                dep = epi(i - 1, p, tprev)
            tprev = t[:16]
        acc_v[i % 2] = acc
        if with_epi:
            epi_done(i - 1)

    def d_body(i, carry):
        d_step(i, True)
        return carry

    d_step(0, False)
    jax.lax.fori_loop(1, NQ, d_body, 0)
    for u in range(NP):
        epi(NQ - 1, u)
    epi_done(NQ - 1)

    r = jnp.concatenate([r_v[i] for i in range(NQ)], axis=1)
    tok = jax.lax.broadcasted_iota(jnp.int32, (8, S), 1)
    m1 = jnp.max(r, axis=1, keepdims=True)
    i1v = jnp.min(jnp.where(r == m1, tok, S), axis=1, keepdims=True)
    r2 = jnp.where(tok == i1v, -jnp.inf, r)
    m2 = jnp.max(r2, axis=1, keepdims=True)
    i2v = jnp.min(jnp.where(r2 == m2, tok, S), axis=1, keepdims=True)
    i1 = jnp.clip(jnp.max(i1v), 0, S - 1)
    i2 = jnp.clip(jnp.max(i2v), 0, S - 1)
    g1 = pl.multiple_of((i1 // 16) * 16, 16)
    g2 = pl.multiple_of((i2 // 16) * 16, 16)
    rid = jax.lax.broadcasted_iota(jnp.int32, (16, 1), 0)
    grp = [xn_v[pl.ds(g1, 16), :].astype(f32), xn_v[pl.ds(g2, 16), :].astype(f32)]
    t1 = jnp.sum(jnp.where(rid + g1 == i1, grp[0], 0.0), axis=0, keepdims=True)
    t2 = jnp.sum(jnp.where(rid + g2 == i2, grp[1], 0.0), axis=0, keepdims=True)
    xs = jnp.where(rid == 0, t1, jnp.where(rid == 1, t2, 0.0)).astype(bf16)
    for c in big[1:]:
        c.wait()
    g = _rb(_mm(xs, wg_v[...]))
    g = _rb(g * _rb(jax.nn.sigmoid(g)))
    u = _rb(_mm(xs, wu_v[...]))
    a = (g * u).astype(bf16)
    FH = F // 2
    y = _rb(_mm(a[:, :FH], wd_v[:FH, :]) + _mm(a[:, FH:], wd_v[FH:, :]))
    y1 = _rb(y[0:1] * _rb(jax.nn.sigmoid(m1[0:1, :])))
    y2 = _rb(y[1:2] * _rb(jax.nn.sigmoid(m2[0:1, :])))
    for n, gbase in enumerate((g1, g2)):
        upd = jnp.where(rid + gbase == i1, y1, 0.0) + jnp.where(rid + gbase == i2, y2, 0.0)
        hh_ = x_v[pl.ds(gbase, 16), :].astype(f32)
        pt_v[n] = (hh_ + _rb(grp[n] + upd)).astype(bf16)
    for i in range(NQ):
        o_copy(i).wait()
    cp1 = pltpu.make_async_copy(pt_v.at[0], out_hbm.at[pl.ds(g1, 16)], sem_p.at[0])
    cp2 = pltpu.make_async_copy(pt_v.at[1], out_hbm.at[pl.ds(g2, 16)], sem_p.at[1])
    cp1.start()

    @pl.when(g1 != g2)
    def _():
        cp2.start()
        cp2.wait()

    cp1.wait()


@jax.jit
def pallas_sequential_preLN__compressed_kv_cla__moe_arch_mod__prompt_kernel(
        A_x, A_c_kv, A_w_q, A_w_uk, A_w_uv, A_w_o, B_x, B_w_r, B_w_gate, B_w_up, B_w_down):
    any_spec = pl.BlockSpec(memory_space=pl.ANY)
    vmem_spec = pl.BlockSpec(memory_space=pltpu.VMEM)
    out = pl.pallas_call(
        _kernel,
        out_shape=jax.ShapeDtypeStruct((S, M), bf16),
        in_specs=[any_spec] * 6 + [vmem_spec] + [any_spec] * 3,
        out_specs=any_spec,
        scratch_shapes=[
            pltpu.VMEM((S, M), bf16),
            pltpu.VMEM((S, DC), bf16),
            pltpu.VMEM((4, CH, D), bf16),
            pltpu.VMEM((NP, 2 * D, M), bf16),
            pltpu.VMEM((M, F), bf16),
            pltpu.VMEM((M, F), bf16),
            pltpu.VMEM((F, M), bf16),
            pltpu.VMEM((NP, 2 * DC + M, 2 * D), bf16),
            pltpu.VMEM((S, M), bf16),
            pltpu.VMEM((BQ, 2 * D), bf16),
            pltpu.VMEM((S, 2 * D), bf16),
            pltpu.VMEM((NP, S, 2 * D), bf16),
            pltpu.VMEM((S, 2 * D), bf16),
            pltpu.VMEM((NP, S, 2 * D), bf16),
            pltpu.VMEM((2, BQ, M), f32),
            pltpu.VMEM((S, M), bf16),
            pltpu.VMEM((NQ, 8, BQ), f32),
            pltpu.VMEM((2, 16, M), bf16),
            pltpu.SemaphoreType.DMA((S // TC,)),
            pltpu.SemaphoreType.DMA((S // LR,)),
            pltpu.SemaphoreType.DMA((4,)),
            pltpu.SemaphoreType.DMA((4,)),
            pltpu.SemaphoreType.DMA((NQ,)),
            pltpu.SemaphoreType.DMA((2,)),
        ],
        compiler_params=pltpu.CompilerParams(vmem_limit_bytes=120 * 1024 * 1024),
    )(A_x.reshape(S, M), A_c_kv.reshape(S, DC), A_w_q.reshape(M * H, D),
      A_w_uk.reshape(DC * H, D), A_w_uv.reshape(DC * H, D), A_w_o.reshape(NP, 2 * D, M),
      B_w_r, B_w_gate, B_w_up, B_w_down)
    return out.reshape(1, S, M)
```
